```python
import os as _os
_os.environ.setdefault("JAX_PLATFORMS", "cpu")
import jax
import jax.numpy as jnp

def _softmax(x, axis=-1):
    return jax.nn.softmax(x, axis=axis)
def _gelu(x):
    return jax.nn.gelu(x, approximate=True)
def _silu(x):
    return jax.nn.silu(x)
def _sigmoid(x):
    return jax.nn.sigmoid(x)
def _layernorm(x, axis=-1, eps=1e-5):
    m = jnp.mean(x, axis=axis, keepdims=True)
    v = jnp.var(x, axis=axis, keepdims=True)
    return (x - m) / jnp.sqrt(v + eps)
def _scatter_add(tgt, idx, src, axis=0):
    return tgt.at[idx].add(src)
def _segment_sum(src, seg, n):
    return jax.ops.segment_sum(src, seg, n)
class _Rng:
    def __init__(self, key):
        self._k = key
    def _next(self):
        self._k, sub = jax.random.split(self._k)
        return sub
    def normal(self, shape):
        return jax.random.normal(self._next(), shape, dtype=jnp.bfloat16)
    def randint(self, lo, hi, shape):
        return jax.random.randint(self._next(), shape, lo, hi, dtype=jnp.int32)
    def uniform(self, shape, lo=0.0, hi=1.0):
        return jax.random.uniform(self._next(), shape, jnp.bfloat16, lo, hi)
    def permutation(self, n):
        return jax.random.permutation(self._next(), n)


kernel_name = 'concat_heads__gqa_block_cached__mha_block_cached__near_ridge'

def setup_inputs():
    _rng = _Rng(jax.random.key(int.from_bytes(__import__("os").urandom(4), "little")))
    _w = (lambda a: (lambda t: t.astype(jnp.bfloat16) if jnp.issubdtype(t.dtype, jnp.floating) else t)(jnp.asarray(a)))
    def _A_setup():
        B, Sq, D = 8, 224, 512
        Hq, Hkv, Sk, Dh = 32, 32, 512, 128
        assert Hq % Hkv == 0, (Hq, Hkv)
        return {
            "x": _w((lambda *s: _rng.normal(s) * 0.8)(B, Sq, D)),
            "k_cache": _w((lambda *s: _rng.normal(s) * 0.8)(B, Hkv, Sk, Dh)),
            "v_cache": _w((lambda *s: _rng.normal(s) * 0.05)(B, Hkv, Sk, Dh)),
            "wq": _w((lambda *s: _rng.normal(s) * 0.8)(D, Hq * Dh) * (D ** -0.5)),
            "wo": _w((lambda *s: _rng.normal(s) * 0.05)(Hq * Dh, D) * ((Hq * Dh) ** -0.5)),
        }
    _A_in = _A_setup()

    def _B_setup():
        B, Sq, D = 8, 224, 512
        H, Sk, Dh = 32, 512, 128
        return {
            "x": _w((lambda *s: _rng.normal(s) * 0.8)(B, Sq, D)),
            "k_cache": _w((lambda *s: _rng.normal(s) * 0.8)(B, H, Sk, Dh)),
            "v_cache": _w((lambda *s: _rng.normal(s) * 0.05)(B, H, Sk, Dh)),
            "wq": _w((lambda *s: _rng.normal(s) * 0.8)(D, H * Dh) * (D ** -0.5)),
            "wo": _w((lambda *s: _rng.normal(s) * 0.05)(H * Dh, D) * ((H * Dh) ** -0.5)),
        }
    _B_in = _B_setup()

    return {
        "A_x": _A_in["x"],
        "A_k_cache": _A_in["k_cache"],
        "A_v_cache": _A_in["v_cache"],
        "A_wq": _A_in["wq"],
        "A_wo": _A_in["wo"],
        "B_x": _B_in["x"],
        "B_k_cache": _B_in["k_cache"],
        "B_v_cache": _B_in["v_cache"],
        "B_wq": _B_in["wq"],
        "B_wo": _B_in["wo"],
    }

def reference(A_x, A_k_cache, A_v_cache, A_wq, A_wo, B_x, B_k_cache, B_v_cache, B_wq, B_wo):
    def _A_ref(x, k_cache, v_cache, wq, wo):
        B, Sq, D = x.shape
        Hq, Dh = 32, 128
        Hkv = k_cache.shape[1]
        rep = Hq // Hkv
        q = (lambda x, *d: x.transpose(*d))((x @ wq).reshape(B, Sq, Hq, Dh), 0, 2, 1, 3)
        k = jnp.repeat(k_cache, rep, axis=1)
        v = jnp.repeat(v_cache, rep, axis=1)
        scores = jnp.einsum("bhqd,bhkd->bhqk", q, k) * (Dh ** -0.5)
        p = _softmax(scores, axis=-1)
        o = jnp.einsum("bhqk,bhkd->bhqd", p, v)
        return (lambda x, *d: x.transpose(*d))(o, 0, 2, 1, 3).reshape(B, Sq, Hq * Dh) @ wo

    def _B_ref(x, k_cache, v_cache, wq, wo):
        B, Sq, D = x.shape
        H, Dh = 32, 128
        q = (lambda x, *d: x.transpose(*d))((x @ wq).reshape(B, Sq, H, Dh), 0, 2, 1, 3)
        scores = jnp.einsum("bhqd,bhkd->bhqk", q, k_cache) * (Dh ** -0.5)
        p = _softmax(scores, axis=-1)
        o = jnp.einsum("bhqk,bhkd->bhqd", p, v_cache)
        return (lambda x, *d: x.transpose(*d))(o, 0, 2, 1, 3).reshape(B, Sq, H * Dh) @ wo

    a = _A_ref(A_x, A_k_cache, A_v_cache, A_wq, A_wo)
    b = _B_ref(B_x, B_k_cache, B_v_cache, B_wq, B_wo)
    return jnp.concatenate([a, b], axis=-1)
```

```python
import functools
import jax
import jax.numpy as jnp
from jax import lax
import jax.experimental.pallas as pl
import jax.experimental.pallas.tpu as pltpu

B, SQ, D, H, SK, DH = 8, 224, 512, 32, 512, 128
LOG2E = 1.4426950408889634
F32, BF16 = jnp.float32, jnp.bfloat16
NT = (((1,), (1,)), ((), ()))


def make(G=4, NB=1, NBUF=2, lag=1):
    NG = H // G
    NBB = B // NB
    NIT = NG * NBB

    def kernel(ax, ak, av, awq, awo, bx, bk, bv, bwq, bwo, out_hbm,
               x_buf, wq_buf, wo_buf, k_buf, v_buf, acc, obuf, x_sem, w_sem, kv_sem, o_sem):
        xs, ks, vs, wqs, wos = (ax, bx), (ak, bk), (av, bv), (awq, bwq), (awo, bwo)

        def kv_copy(it, br, j, which):
            g = it // NBB
            b = (it % NBB) * NB + j
            slot = it % NBUF
            src, dst = (ks, k_buf) if which == 0 else (vs, v_buf)
            return pltpu.make_async_copy(src[br].at[b, pl.ds(g * G, G)], dst.at[slot, br, j], kv_sem.at[slot, br, j, which])

        def w_copy(g, br, which):
            slot = g % 2
            c0 = pl.multiple_of(g * (G * DH), G * DH)
            if which == 0:
                return pltpu.make_async_copy(wqs[br].at[:, pl.ds(c0, G * DH)], wq_buf.at[slot, br], w_sem.at[slot, br, 0])
            return pltpu.make_async_copy(wos[br].at[pl.ds(c0, G * DH), :], wo_buf.at[slot, br], w_sem.at[slot, br, 1])

        def x_copy(br, b):
            return pltpu.make_async_copy(xs[br].at[b], x_buf.at[br, b], x_sem.at[br, b])

        def o_copy(br, b):
            return pltpu.make_async_copy(obuf.at[br, b], out_hbm.at[b, :, pl.ds(br * D, D)], o_sem.at[br, b])

        for j in range(NB):
            for br in range(2):
                x_copy(br, j).start()
                if j == 0:
                    w_copy(0, br, 0).start()
                kv_copy(0, br, j, 0).start()
                kv_copy(0, br, j, 1).start()
                if j == 0:
                    w_copy(0, br, 1).start()
        for it in range(1, NBUF - 1):
            for j in range(NB):
                for br in range(2):
                    kv_copy(it, br, j, 0).start()
                    kv_copy(it, br, j, 1).start()
        for b in range(NB, B):
            for br in range(2):
                x_copy(br, b).start()
        acc[...] = jnp.zeros(acc.shape, F32)

        def body(it, carry):
            g = it // NBB
            bb = it % NBB
            slot = it % NBUF
            ws = g % 2
            nxt = it + NBUF - 1

            @pl.when(nxt < NIT)
            def _():
                for j in range(NB):
                    for br in range(2):
                        kv_copy(nxt, br, j, 0).start()
                        kv_copy(nxt, br, j, 1).start()

            @pl.when(bb == 0)
            def _():
                @pl.when(g + 1 < NG)
                def _():
                    for br in range(2):
                        w_copy(g + 1, br, 0).start()
                        w_copy(g + 1, br, 1).start()
                for br in range(2):
                    w_copy(g, br, 0).wait()
                    w_copy(g, br, 1).wait()

            @pl.when(g == 0)
            def _():
                for j in range(NB):
                    for br in range(2):
                        x_copy(br, bb * NB + j).wait()

            for j in range(NB):
                for br in range(2):
                    kv_copy(it, br, j, 0).wait()
                    kv_copy(it, br, j, 1).wait()
            units = [(j, br, h) for j in range(NB) for br in range(2) for h in range(G)]
            q, p, l, o = {}, {}, {}, {}

            def do_q(u):
                j, br, h = u
                r = jnp.dot(x_buf[br, bb * NB + j], wq_buf[ws, br, :, h * DH:(h + 1) * DH], preferred_element_type=F32)
                q[u] = (r * (DH ** -0.5 * LOG2E)).astype(BF16)

            def do_s(u):
                j, br, h = u
                s = lax.dot_general(q.pop(u), k_buf[slot, br, j, h], NT, preferred_element_type=F32)
                m = jnp.max(s, axis=-1, keepdims=True)
                e = jnp.exp2(s - m)
                l[u] = jnp.sum(e, axis=-1, keepdims=True)
                p[u] = e.astype(BF16)

            def do_pv(u):
                j, br, h = u
                r = jnp.dot(p.pop(u), v_buf[slot, br, j, h], preferred_element_type=F32)
                ll = l.pop(u)
                r0 = pl.reciprocal(ll, approx=True)
                r0 = r0 * (2.0 - ll * r0)
                o[u] = (r * r0).astype(BF16)

            def do_o(u):
                j, br, h = u
                assert G == 4
                oo = jnp.concatenate([o[(j, br, hh)] for hh in range(G)], axis=-1)
                b = bb * NB + j
                cs = slice(h * DH, (h + 1) * DH)
                r = acc[br, b, :, cs] + jnp.dot(oo, wo_buf[ws, br, :, cs], preferred_element_type=F32)
                acc[br, b, :, cs] = r
                obuf[br, b, :, cs] = r.astype(BF16)

            n = len(units)
            for t in range(n + 2 * lag + G + 1):
                if t < n:
                    do_q(units[t])
                if 0 <= t - lag < n:
                    do_s(units[t - lag])
                if 0 <= t - 2 * lag < n:
                    do_pv(units[t - 2 * lag])
                if 0 <= t - 2 * lag - G < n:
                    do_o(units[t - 2 * lag - G])

            @pl.when(g == NG - 1)
            def _():
                for j in range(NB):
                    for br in range(2):
                        o_copy(br, bb * NB + j).start()
            return carry

        lax.fori_loop(0, NIT, body, 0)
        for b in range(B):
            for br in range(2):
                o_copy(br, b).wait()

    any_spec = pl.BlockSpec(memory_space=pl.ANY)

    @jax.jit
    def fn(*args):
        return pl.pallas_call(
            kernel,
            in_specs=[any_spec] * 10,
            out_specs=any_spec,
            out_shape=jax.ShapeDtypeStruct((B, SQ, 2 * D), BF16),
            scratch_shapes=[
                pltpu.VMEM((2, B, SQ, D), BF16),
                pltpu.VMEM((2, 2, D, G * DH), BF16),
                pltpu.VMEM((2, 2, G * DH, D), BF16),
                pltpu.VMEM((NBUF, 2, NB, G, SK, DH), BF16),
                pltpu.VMEM((NBUF, 2, NB, G, SK, DH), BF16),
                pltpu.VMEM((2, B, SQ, D), F32),
                pltpu.VMEM((2, B, SQ, D), BF16),
                pltpu.SemaphoreType.DMA((2, B)),
                pltpu.SemaphoreType.DMA((2, 2, 2)),
                pltpu.SemaphoreType.DMA((NBUF, 2, NB, 2)),
                pltpu.SemaphoreType.DMA((2, B)),
            ],
            compiler_params=pltpu.CompilerParams(vmem_limit_bytes=110 * 1024 * 1024),
        )(*args)
    return fn


_fn = None


@jax.jit
def pallas_concat_heads__gqa_block_cached__mha_block_cached__near_ridge_kernel(
    A_x, A_k_cache, A_v_cache, A_wq, A_wo, B_x, B_k_cache, B_v_cache, B_wq, B_wo):
    return make(G=4, NB=2)(A_x, A_k_cache, A_v_cache, A_wq, A_wo, B_x, B_k_cache, B_v_cache, B_wq, B_wo)
```

```python
import functools, contextlib
import jax
import jax.numpy as jnp
from jax import lax
import jax.experimental.pallas as pl
import jax.experimental.pallas.tpu as pltpu

B, SQ, D, H, SK, DH = 8, 224, 512, 32, 512, 128
G = 8
NG = H // G
LOG2E = 1.4426950408889634
F32, BF16, U32 = jnp.float32, jnp.bfloat16, jnp.uint32
NT = (((1,), (1,)), ((), ()))
T = ((1, 0), (0, 1), (-1, 0), (0, -1))
ORDER = ((0, 1), (1, 0), (0, 0), (1, 1))


def lin(*terms):
    terms = sorted([t for t in terms if t[0]], key=lambda t: t[0] < 0)
    assert terms[0][0] > 0
    r = None
    for c, v in terms:
        if abs(c) != 1:
            v = v * float(abs(c))
        r = v if r is None else (r + v if c > 0 else r - v)
    return r


def add_rows_times(base, z, t):
    c, d = t
    return lambda a, e: lin((1, base(a, e)), (c, c and z(a, e)), (d if e else -d, d and z(a, 1 - e)))


def add_times_cols(base, t, z):
    c, d = t
    return lambda e, b: lin((1, base(e, b)), (c, c and z(e, b)), (-d if e else d, d and z(1 - e, b)))


def gsum(*terms):
    return lambda a, b: lin(*[(c, g(a, b)) for c, g in terms])


def fixed(grid):
    vals = [[grid(a, b) for b in range(2)] for a in range(2)]
    return lambda a, b: vals[a][b]


def strassen_lhs(x):
    return (lambda: x(0, 0), lambda: x(0, 0) + x(0, 1), lambda: x(1, 0) + x(1, 1), lambda: x(1, 1),
            lambda: x(0, 0) + x(1, 1), lambda: x(0, 1) - x(1, 1), lambda: x(1, 0) - x(0, 0))


def strassen_rhs(w, flip):
    y = (lambda e, b: w(e, 1 - b)) if flip else w
    yield y(0, 1) - y(1, 1)
    yield y(1, 1)
    yield y(0, 0)
    yield y(1, 0) - y(0, 0)
    yield y(0, 0) + y(1, 1)
    yield y(1, 0) + y(1, 1)
    yield y(0, 0) + y(0, 1)


def strassen(lhs, flip):
    ms = []
    for f in lhs:
        ms.append((yield f))
    m3, m5, m2, m4, m1, m7, m6 = ms
    c12, c21 = m3 + m5, m2 + m4
    c = [[((m4 - m5) + m1) + m7, c12], [c21, ((m3 - m2) + m1) + m6]]
    return lambda a, b: c[a][b ^ flip]


PAIRS = [(i, j) for i in range(4) for j in range(i + 1, 4)]
BLOCKS = ((0, 1), (1, 0), (0, 2), (2, 0), (0, 3), (3, 0), (0, 0), (1, 2), (2, 1), (1, 3), (3, 1), (1, 1), (2, 3), (3, 2), (2, 2), (3, 3))
ACC = [(1, i, j) for i in range(4) for j in range(4)] + [(0, i, j) for i in range(4) for j in range(i, 4)]
O_READY = (0, 1, 3, 4, 6, 7, 9, 11, 12, 14, 15, 17, 19, 20, 22, 24, 26)


def make_plan(lo=6, hi=66, pos=2):
    out, no, done = [], 0, 0
    for t in range(65):
        r = ""
        while done < 45 and (t - lo) * 42 >= done * (hi - lo) and no + 4 <= 7 * O_READY[max(t - 2, 0) // 4] and not r:
            r, no, done = "0", no + 4, done + 1
        out.append("S" * (t < 64) + r * (pos == 1) + "P" * (t >= 1) + r * (pos == 2))
    return "".join(out) + "0" * (45 - done) + "h"


def make(nobc=True, flags={"XLA_TPU_RESCHEDULE_DMA_DONES": True}, nz=3, bkeep=True, plan=None, prof=False, pad=8, xkeep='bu', early=((1, 3, (1, 3, 2)), (0, 3, (0, 1, 3)), (1, 2, (1, 2, 3))), nosem=True, qwait=(0, 24, 88, 200, 360), qlag=0, parts='qa', qplan='0001' + '11110000' * 44 + '1111' + '0001',
         fastld=True):
    plan = plan or make_plan()
    scope = jax.named_scope if prof else (lambda n: contextlib.nullcontext())

    def ld(ref):
        return pltpu.bitcast(ref.bitcast(U32)[...], BF16) if fastld else ref[...]

    def kernel(ax, ak, av, awq, awo, bx, bk, bv, bwq, bwo, out_hbm,
               q_buf, k_buf, v_buf, out_buf, acc, sem, out_sem, *bufs):
        o_bufs, d_bufs = dict(zip([n for n, b in enumerate(BLOCKS) if b[0] != b[1]], bufs)), bufs[12:]
        x_bufs, wq_bufs, wo_bufs = bufs[20:24], (bufs[24:28], bufs[28:32]), bufs[32:36]
        xs, ks, vs, wqs, wos = (ax, bx), (ak, bk), (av, bv), (awq, bwq), (awo, bwo)

        def kv_copy(br, job, n, which):
            src, dst = (ks, k_buf) if which == 0 else (vs, v_buf)
            i, j = BLOCKS[n]
            return pltpu.make_async_copy(src[br].at[pl.ds(2 * i, 2), pl.ds((job & 3) * G + 2 * j, 2)], dst.at[n], sem.at[2 * n + which])

        def wq_copy(br, job, u, j):
            c0 = pl.multiple_of((((job & 3) + u) * G + 2 * j) * DH, 2 * DH)
            return pltpu.make_async_copy(wqs[br].at[:, pl.ds(c0, 2 * DH)], wq_bufs[u][j].at[(job >> 1) & 1], sem.at[44 + 4 * u + j])

        def wo_copy(br, job, j):
            c0 = pl.multiple_of(((job & 3) * G + 2 * j) * DH, 2 * DH)
            return pltpu.make_async_copy(wos[br].at[pl.ds(c0, 2 * DH), :], wo_bufs[j].at[job & 1], sem.at[36 + j])

        def x_copy(br, i):
            return pltpu.make_async_copy(xs[br].at[pl.ds(2 * i, 2)], x_bufs[i].at[0], sem.at[40 + i])

        def out_copy(br, i, e):
            cols = pl.ds(pl.multiple_of(br * D + e * DH, DH), DH)
            return pltpu.make_async_copy(out_buf.at[br, e, pl.ds(2 * i, 2)], out_hbm.at[pl.ds(2 * i, 2), :, cols], out_sem.at[br, e])

        def prefetch(job, copy, *args):
            for br in range(2):
                pl.when((job >> 2) == br)(lambda br=br: copy(br, job, *args).start())

        first_w = {0: (0, 1), 1: (2,), 3: (3,)}

        def body(job, carry):
            br, g, slot = job >> 2, job & 3, job & 1
            q, o_done = {}, set()
            now = {"round": 0}

            def zero():
                return job >> (3 + now["round"] % nz)

            def wait(copy, *args):
                copy(0, job, *args).wait()

            def q_weights(u):
                ga = {}
                wt = lambda j, e0: lambda e, h: wq_bufs[u][j][((job >> 1) & 1) + zero(), (e0 + e) * DH:(e0 + e + 1) * DH, h * DH:(h + 1) * DH].astype(F32)
                for j in range(4):
                    yield from strassen_rhs(wt(j, 2), 1)
                    ga[j] = fixed(add_times_cols(wt(j, 0), (-T[j][0], -T[j][1]), wt(j, 2)))
                    yield from strassen_rhs(ga[j], 0)
                    for i in range(j):
                        c, d = T[j][0] - T[i][0], T[j][1] - T[i][1]
                        z = fixed(gsum((1, ga[i]), (1, ga[j])))
                        if c and d:
                            t = fixed(lambda e, h: lin((1, z(e, h)), (c * d if e else -c * d, z(1 - e, h))) * (0.5 * c))
                        else:
                            t = fixed(lambda e, h: z(e, h) * (1 / c) if c else z(1 - e, h) * (1 / d if e else -1 / d))
                        yield from strassen_rhs(t, 1)
                        yield from strassen_rhs(gsum((1, t), (1, wt(j, 2))), 0)
                        yield from strassen_rhs(gsum((1, t), (-1, wt(i, 2))), 0)

            def x_operands():
                be = {}
                xt = lambda j, e0: lambda a, e: x_bufs[j][zero(), a, :, (e0 + e) * DH:(e0 + e + 1) * DH].astype(F32)
                keep = lambda grid, k: fixed(grid) if k in xkeep else grid
                for j in range(4):
                    be[j] = keep(add_rows_times(xt(j, 2), xt(j, 0), T[j]), "b")
                    yield from strassen_lhs(be[j])
                    yield from strassen_lhs(xt(j, 0))
                    for i in range(j):
                        c, d = T[j][0] - T[i][0], T[j][1] - T[i][1]
                        s = keep(gsum((1, be[i]), (1, be[j])), "s")
                        yield from strassen_lhs(s)
                        yield from strassen_lhs(keep(add_rows_times(s, xt(i, 0), (c, d)), "u"))
                        yield from strassen_lhs(keep(add_rows_times(s, xt(j, 0), (-c, -d)), "u"))

            def q_proj(u, operand):
                pp, qq = {}, {}
                group = iter(range(26))
                lhs = lambda: [functools.partial(operand, 7 * n + k) for n in [next(group)] for k in range(7)]

                def emit(i, j, c):
                    for a, h in ORDER:
                        q_buf[u, 2 * i + a, 2 * j + h] = (c(a, h) * (DH ** -0.5 * LOG2E)).astype(BF16)
                for j in range(4):
                    qq[j] = yield from strassen(lhs(), 1)
                    pp[j] = yield from strassen(lhs(), 0)
                    emit(j, j, gsum((1, pp[j]), (1, qq[j])))
                    for i in range(j):
                        r = yield from strassen(lhs(), 1)
                        m = yield from strassen(lhs(), 0)
                        emit(i, j, gsum((1, m), (-1, r), (-1, pp[i]), (-1, qq[j])))
                        v = yield from strassen(lhs(), 0)
                        emit(j, i, gsum((1, r), (-1, v), (-1, pp[j]), (-1, qq[i])))

            def o_weights():
                be = {}
                wt = lambda j, e0: lambda h, e: wo_bufs[j][slot + zero(), h * DH:(h + 1) * DH, (e0 + e) * DH:(e0 + e + 1) * DH].astype(F32)

                def diag(i):
                    yield from strassen_rhs(gsum((2, wt(i, 0))), 0)
                    yield from strassen_rhs(be[i], 1)
                for i, j in PAIRS:
                    for k in (i, j):
                        if k not in be:
                            be[k] = add_rows_times(wt(k, 2), wt(k, 0), T[k])
                            if bkeep:
                                be[k] = fixed(be[k])
                    c, d = T[j][0] - T[i][0], T[j][1] - T[i][1]
                    flip = (i + j) & 1
                    s = fixed(gsum((1, be[i]), (1, be[j])))
                    yield from strassen_rhs(add_rows_times(s, wt(j, 0), (-c, -d)), flip)
                    yield from strassen_rhs(add_rows_times(s, wt(i, 0), (c, d)), flip)
                    yield from strassen_rhs(s, 1 - flip)
                    if j == 3:
                        yield from diag(i)
                yield from diag(3)

            def o_proj():
                o = lambda i, j: lambda a, h: o_bufs[BLOCKS.index((i, j))][zero(), a, h, 0:SQ]
                stored = lambda *key: lambda a, e: acc[a, e, ACC.index(key), 0:SQ]

                def save(key, m):
                    vals = [(k, m(*k)) for k in ORDER]
                    for (a, e), v in vals:
                        acc[a, e, ACC.index(key), 0:SQ] = v
                    return dict(vals)

                pending = {(which, i): [] for which in range(2) for i in range(4)}
                started = set()

                def fold(which, i, *terms):
                    m = stored(which, i, i)
                    if (which, i) not in started:
                        started.add((which, i))
                        m = lambda a, e: jnp.where(g == 0, 0.0, stored(which, i, i)(a, e))
                    for part, t in list(terms) + pending[which, i]:
                        m = add_rows_times(m, part, t)
                    pending[which, i] = []
                    return save((which, i, i), m)

                def contribute(which, i, key, vals, t):
                    if (which, i, key) in early:
                        fold(which, i, (lambda a, e: vals[a, e], t))
                    else:
                        pending[which, i].append((stored(*key), t))

                def diag(i, which):
                    yield [k for k in BLOCKS if k[1 - which] == i]
                    m = yield from strassen(strassen_lhs(lambda a, h: d_bufs[2 * i + which][zero(), a, h, 0:SQ]), which)
                    if which == 0:
                        res = {k: v * 0.5 for k, v in fold(0, i, (m, (1, 0))).items()}
                    else:
                        c, d = T[i]
                        lo = {(a, e): stored(0, i, i)(a, e if c else 1 - e) * (-0.5 * (c or (d if e else -d))) for a, e in ORDER}
                        res = {k: v + lo[k] for k, v in fold(1, i, (m, (1, 0))).items()}
                    for (a, e), v in res.items():
                        out_buf[br, 2 * which + e, 2 * i + a] = v.astype(BF16)
                    for e in range(2):
                        pl.when(g == NG - 1)(lambda: out_copy(br, i, 2 * which + e).start())

                for i, j in PAIRS:
                    c, d = T[j][0] - T[i][0], T[j][1] - T[i][1]
                    flip = (i + j) & 1
                    for r, k in ((i, j), (j, i)):
                        yield [(r, k)]
                        m = yield from strassen(strassen_lhs(o(r, k)), flip)
                        contribute(1, r, (1, r, k), save((1, r, k), m), (1, 0))
                    m = yield from strassen(strassen_lhs(gsum((1, o(i, j)), (-1, o(j, i)))), 1 - flip)
                    vals = save((0, i, j), gsum((1, m), (1, stored(1, j, i)), (-1, stored(1, i, j))))
                    for k in (i, j):
                        contribute(0, k, (0, i, j), vals, (c, -d) if c and d else (c // 2, -d // 2))
                    if j == 3:
                        yield from diag(i, 0)
                        yield from diag(i, 1)
                yield from diag(3, 0)
                yield from diag(3, 1)

            class Stream:
                def __init__(self, gen, weights):
                    self.gen, self.weights = gen, weights
                    self.next = next(gen)

                def step(self, pieces=1):
                    while isinstance(self.next, list):
                        assert all(k in o_done for k in self.next)
                        self.next = next(self.gen)
                    a, w = self.next(), next(self.weights)
                    w, c = w.astype(BF16), SQ // pieces
                    m = [jnp.dot((a if pieces == 1 else a[i:i + c]).astype(BF16), w, preferred_element_type=F32) for i in range(0, SQ, c)]
                    try:
                        self.next = self.gen.send(jnp.concatenate(m, axis=0))
                    except StopIteration:
                        self.next = None

            def q_phase():
                gen, made = x_operands(), []

                def operand(n):
                    if n == len(made):
                        made.append(next(gen)().astype(BF16))
                    return made[n]
                qs = [Stream(q_proj(u, operand), q_weights(u)) for u in range(2)]
                for n, ch in enumerate(qplan):
                    now["round"] = n // 4
                    if n in qwait:
                        j = qwait.index(n)
                        for u in range(2):
                            if j:
                                prefetch(job + 2, wq_copy, u, j - 1)
                        if j < 4:
                            pl.when(g == 0)(lambda: x_copy(0, j).wait())
                            wait(wq_copy, 0, j)
                    if n - qlag in qwait[:4]:
                        wait(wq_copy, 1, qwait.index(n - qlag))
                    qs[int(ch)].step()
                assert qs[0].next is None and qs[1].next is None

            with scope("q"):
                if "q" in parts:
                    pl.when(slot == 0)(q_phase)
            if "a" not in parts:
                out_buf[0, 0] = q_buf[slot, :, job]
                out_copy(0, 0, 0).start()
                return carry
            os_ = Stream(o_proj(), o_weights())
            HS = SQ // 2
            p, l, r = {}, {}, {}

            pk = [k for ch in plan if ch in 'Pp' for k in ((2, 2) if ch == 'P' else (1,))]

            def unit(t, k):
                assert k == 1 or t % 2 == 0
                return (t // 8,) + ORDER[t // 2 % 4] + (t % 2 * HS, (t % 2 + k) * HS)

            def cat(d, t, k):
                return jnp.concatenate([d[t + i] for i in range(k)], axis=0)

            def do_s(t, k, tie):
                n, a, h, lo, hi = unit(t, k)
                i, j = BLOCKS[n]
                if t % 8 == 0:
                    wait(kv_copy, n, 0)
                s = lax.dot_general(ld(q_buf.at[slot, 2 * i + a, 2 * j + h, lo:hi]), ld(k_buf.at[n, a, h]), NT, preferred_element_type=F32)
                if (t + k) % 8 == 0:
                    prefetch(job + 1, kv_copy, n, 0)
                e = jnp.exp2(s - jnp.max(s, axis=-1, keepdims=True))
                ll = jnp.broadcast_to(jnp.sum(e, axis=-1, keepdims=True), (k * HS, DH))
                rr = pltpu.reciprocal(ll, approx=True)
                for u in range(k):
                    l[t + u], r[t + u] = ll[u * HS:(u + 1) * HS], rr[u * HS:(u + 1) * HS]
                if t - tie in l:
                    e = jnp.concatenate([e[:, :3 * DH], jnp.minimum(e[:, 3 * DH:], cat(l, t - tie, k))], axis=-1)
                if pk[t] == k:
                    p[t] = e.astype(BF16)
                elif k == 2:
                    p[t], p[t + 1] = e[:HS].astype(BF16), e[HS:].astype(BF16)
                elif t % 2 == 0:
                    p[t] = e
                else:
                    p[t - 1] = jnp.concatenate([p[t - 1], e], axis=0).astype(BF16)

            def do_pv(t, k):
                n, a, h, lo, hi = unit(t, k)
                if t % 8 == 0:
                    wait(kv_copy, n, 1)
                    for j in first_w.get(n, []):
                        wait(wo_copy, j)
                        prefetch(job + 1, wo_copy, j)
                o = jnp.dot(p.pop(t), ld(v_buf.at[n, a, h]), preferred_element_type=F32)
                if (t + k) % 8 == 0:
                    prefetch(job + 1, kv_copy, n, 1)
                    o_done.add(BLOCKS[n])
                o = o * cat(r, t, k)
                if n in o_bufs:
                    o_bufs[n][0, a, h, lo:hi] = o
                for which in range(2):
                    i = BLOCKS[n][1 - which]
                    line = [b for b in BLOCKS if b[1 - which] == i]
                    if line[-1] == BLOCKS[n]:
                        d_bufs[2 * i + which][0, a, h, lo:hi] = lin(
                            *[(1 if b == (i, i) else -1, o if b == BLOCKS[n] else o_bufs[BLOCKS.index(b)][zero(), a, h, lo:hi]) for b in line])

            ns = npv = 0
            for ch in plan:
                now["round"] += 1
                k = 2 if ch.isupper() else 1
                if ch in "SsTtUu":
                    do_s(ns, k, {"s": 2, "t": 1, "u": 0}[ch.lower()])
                    ns += k
                elif ch in "Pp":
                    do_pv(npv, k)
                    npv += k
                else:
                    for i in range(4 if ch == "0" else 2):
                        os_.step(1 if ch == "0" else 2)
            assert os_.next is None and ns == npv == 128
            for j in range(4):
                pl.when(job == 2)(lambda: x_copy(1, j).start())
            return carry

        for j in range(4):
            x_copy(0, j).start()
            wq_copy(0, 0, 0, j).start()
            wq_copy(0, 0, 1, j).start()
        for n in range(16):
            kv_copy(0, 0, n, 0).start()
            kv_copy(0, 0, n, 1).start()
            for j in first_w.get(n, []):
                wo_copy(0, 0, j).start()
        lax.fori_loop(0, 2 * NG, body, 0)
        for br in range(2):
            for e in range(4):
                for i in range(4):
                    out_copy(br, i, e).wait()

    any_spec = pl.BlockSpec(memory_space=pl.ANY)

    @jax.jit
    def fn(*args):
        return pl.pallas_call(
            kernel,
            in_specs=[any_spec] * 10,
            out_specs=any_spec,
            out_shape=jax.ShapeDtypeStruct((B, SQ, 2 * D), BF16),
            scratch_shapes=[
                pltpu.VMEM((2, B, G, SQ, DH), BF16),
                pltpu.VMEM((16, 2, 2, SK, DH), BF16),
                pltpu.VMEM((16, 2, 2, SK, DH), BF16),
                pltpu.VMEM((2, 4, B, SQ, DH), BF16),
                pltpu.VMEM((2, 2, 27, SQ + pad, DH), F32),
                pltpu.SemaphoreType.DMA((52,)),
                pltpu.SemaphoreType.DMA((2, 4)),
            ] + [pltpu.VMEM((1, 2, 2, SQ + pad, DH), F32)] * 20 + [pltpu.VMEM((1, 2, SQ, D), BF16)] * 4 + [pltpu.VMEM((2, D, 2 * DH), BF16)] * 8 + [pltpu.VMEM((2, 2 * DH, D), BF16)] * 4,
            compiler_params=pltpu.CompilerParams(vmem_limit_bytes=110 * 1024 * 1024, disable_bounds_checks=nobc, disable_semaphore_checks=nosem, flags=flags),
        )(*args)
    return fn


@jax.jit
def pallas_concat_heads__gqa_block_cached__mha_block_cached__near_ridge_kernel(
    A_x, A_k_cache, A_v_cache, A_wq, A_wo, B_x, B_k_cache, B_v_cache, B_wq, B_wo):
    return make(plan='$(cat plan19.txt)',qplan='$(cat qplan19.txt)')(A_x, A_k_cache, A_v_cache, A_wq, A_wo, B_x, B_k_cache, B_v_cache, B_wq, B_wo)
```

```python
import functools

import jax
import jax.numpy as jnp
from jax import lax
import jax.experimental.pallas as pl
import jax.experimental.pallas.tpu as pltpu

B, SQ, D, H, SK, DH = 8, 224, 512, 32, 512, 128
G = 8
NG = H // G
HS = SQ // 2
SCALE = DH ** -0.5 * 1.4426950408889634
F32, BF16 = jnp.float32, jnp.bfloat16
NT = (((1,), (1,)), ((), ()))
N_PRODUCTS = 26 * 7
MAX_Q_GROWTH, MAX_OUT_GROWTH = 11.0, 4.0

T = ((1, 0), (0, 1), (-1, 0), (0, -1))
PAIRS = tuple((i, j) for i in range(4) for j in range(i + 1, 4))
QUADS = ((0, 1), (1, 0), (0, 0), (1, 1))
BLOCKS = ((0, 1), (1, 0), (0, 2), (2, 0), (0, 3), (3, 0), (0, 0), (1, 2),
          (2, 1), (1, 3), (3, 1), (1, 1), (2, 3), (3, 2), (2, 2), (3, 3))
SLOTS = (tuple((1, i, j) for i in range(4) for j in range(4))
         + tuple((0, i, j) for i in range(4) for j in range(i, 4)))
SWAPPED = ((0, 0, 0), (0, 2, 2), (0, 0, 1), (0, 0, 2), (0, 1, 3),
           (1, 0, 1), (1, 2, 0), (1, 3, 0), (1, 3, 1))
FOLD_EARLY = ((0, 1, (0, 1, 2)), (1, 1, (1, 1, 3)), (1, 2, (1, 2, 3)), (0, 3, (0, 1, 3)), (1, 3, (1, 3, 2)))
WO_WAIT = {0: (0, 1), 1: (2,), 3: (3,)}
Q_WAIT = (0, 10, 26, 40, 92, 108, 204, 220, 360)

Q_PLAN = (
    "00011111000101110000111100101001010011110000111100001111010001100011001011001111000011110000"
    "11000110101110010011001101110000101111001110000011110000011110010111000011110001010101101011"
    "00001111000011110000111100001111000011101000111100101001001111010010100100011101110011010000"
    "1111001001101000111100001111000110100001111100001111000001111001111000001110110011010100"
)
PLAN = (
    "ssSPPTSPTPpS0SpPSsPpsSpPSP00S0PSPSP0PS0ssP0SPSPS0PSP00SPSSPP00SpSpSppSPPs0s0PS0PSP0P0SSpSpPP"
    "0S0SPS0PSP0SPS0PSPS0P0SPSPSP0SPSP0S0PppS0S0PSP0SP0SPP0SSP0S0PSPSP0SppSP0SP0S0PSP0SP0SPP00000"
    "h"
)


def _lin(*terms):
    terms = sorted([t for t in terms if t[0]], key=lambda t: t[0] < 0)
    total = None
    for c, v in terms:
        if abs(c) != 1:
            v = v * float(abs(c))
        total = v if total is None else (total + v if c > 0 else total - v)
    return total


def _sum(*terms):
    return lambda a, b: _lin(*[(c, grid(a, b)) for c, grid in terms])


def _plus_grid_t(base, z, t):
    c, d = t
    return lambda a, e: _lin((1, base(a, e)), (c, c and z(a, e)), (d if e else -d, d and z(a, 1 - e)))


def _plus_t_grid(base, t, z):
    c, d = t
    return lambda e, b: _lin((1, base(e, b)), (c, c and z(e, b)), (-d if e else d, d and z(1 - e, b)))


def _once(grid):
    vals = [[grid(a, b) for b in range(2)] for a in range(2)]
    return lambda a, b: vals[a][b]


def _tau(i, j):
    return T[j][0] - T[i][0], T[j][1] - T[i][1]


def _strassen_lhs(x):
    return (lambda: x(0, 0), lambda: x(0, 0) + x(0, 1), lambda: x(1, 0) + x(1, 1), lambda: x(1, 1),
            lambda: x(0, 0) + x(1, 1), lambda: x(0, 1) - x(1, 1), lambda: x(1, 0) - x(0, 0))


def _strassen_rhs(w, swap):
    y = (lambda e, b: w(e, 1 - b)) if swap else w
    yield y(0, 1) - y(1, 1)
    yield y(1, 1)
    yield y(0, 0)
    yield y(1, 0) - y(0, 0)
    yield y(0, 0) + y(1, 1)
    yield y(1, 0) + y(1, 1)
    yield y(0, 0) + y(0, 1)


def _strassen(lhs, swap):
    ms = []
    for operand in lhs:
        ms.append((yield operand))
    m3, m5, m2, m4, m1, m7, m6 = ms
    c12, c21 = m3 + m5, m2 + m4
    c = [[((m4 - m5) + m1) + m7, c12], [c21, ((m3 - m2) + m1) + m6]]
    return lambda a, b: c[a][b ^ swap]


def _sample_energy(total, tile, n):
    row = n * 8 % SQ
    v = tile[row:row + 8]
    return v * v if total is None else total + v * v


def _column_sums(v):
    parts = [v[r:r + 8] for r in range(0, v.shape[0], 8)]
    while len(parts) > 1:
        parts = [functools.reduce(jnp.add, parts[i:i + 2]) for i in range(0, len(parts), 2)]
    return jnp.broadcast_to(jnp.sum(parts[0], axis=0, keepdims=True), parts[0].shape)


def _too_large(products, limit):
    return jnp.where((products <= limit) & (limit > 0.0) & (limit < jnp.inf), 0.0, 1.0)


class _Projection:
    def __init__(self, products, weights, done=()):
        self.products, self.weights, self.done = products, weights, done
        self.pending = next(products)
        self.count, self.energy = 0, None

    def step(self, pieces=1):
        while isinstance(self.pending, list):
            assert all(blk in self.done for blk in self.pending)
            self.pending = next(self.products)
        lhs = self.pending()
        rhs = next(self.weights).astype(BF16)
        rows = SQ // pieces
        parts = [jnp.dot((lhs if pieces == 1 else lhs[r:r + rows]).astype(BF16), rhs,
                         preferred_element_type=F32) for r in range(0, SQ, rows)]
        product = jnp.concatenate(parts, axis=0)
        self.energy = _sample_energy(self.energy, product, self.count)
        self.count += 1
        try:
            self.pending = self.products.send(product)
        except StopIteration:
            self.pending = None


def _kernel(ax, ak, av, awq, awo, bx, bk, bv, bwq, bwo, out_hbm,
            q_buf, k_buf, v_buf, out_buf, m_buf, check, plain_buf,
            sem, out_sem, plain_sem, *bufs):
    xs, ks, vs, wqs, wos = (ax, bx), (ak, bk), (av, bv), (awq, bwq), (awo, bwo)
    o_bufs = dict(zip([blk for blk in BLOCKS if blk[0] != blk[1]], bufs))
    out_check, q_check, failed = check.at[0:2], check.at[2], check.at[3, 0]
    d_bufs, x_bufs = bufs[12:20], bufs[20:28]
    wq_bufs, wo_bufs = (bufs[28:32], bufs[32:36]), bufs[36:40]

    def kv_copy(br, job, n, which):
        src, dst = (ks, k_buf) if which == 0 else (vs, v_buf)
        i, j = BLOCKS[n]
        return pltpu.make_async_copy(
            src[br].at[pl.ds(2 * i, 2), pl.ds((job & 3) * G + 2 * j, 2)], dst.at[n], sem.at[2 * n + which])

    def wq_copy(br, job, u, j, half):
        col = pl.multiple_of((((job & 3) + u) * G + 2 * j) * DH, 2 * DH)
        return pltpu.make_async_copy(
            wqs[br].at[pl.ds(half * 2 * DH, 2 * DH), pl.ds(col, 2 * DH)],
            wq_bufs[half][j].at[(job >> 1) & 1, u], sem.at[44 + 4 * j + 2 * half + u])

    def wo_copy(br, job, j):
        row = pl.multiple_of(((job & 3) * G + 2 * j) * DH, 2 * DH)
        return pltpu.make_async_copy(
            wos[br].at[pl.ds(row, 2 * DH), :], wo_bufs[j].at[job & 1], sem.at[32 + j])

    def x_copy(br, b):
        return pltpu.make_async_copy(xs[br].at[b], x_bufs[b].at[0], sem.at[36 + b])

    def out_copy(br, i, e):
        cols = pl.ds(pl.multiple_of(br * D + e * DH, DH), DH)
        return pltpu.make_async_copy(
            out_buf.at[br, e, pl.ds(2 * i, 2)], out_hbm.at[pl.ds(2 * i, 2), :, cols], out_sem.at[br, i, e])

    def prefetch(job, copy, *args):
        for br in range(2):
            pl.when((job >> 2) == br)(lambda br=br: copy(br, job, *args).start())

    def run_job(job, carry):
        br, g, parity = job >> 2, job & 3, job & 1
        position = [0]

        def zero():
            return job >> (3 + position[0] % 3)

        def x_operands():
            beta = {}

            def x_grid(i, e0):
                return lambda a, e: x_bufs[2 * i + a][zero(), :, pl.ds((e0 + e) * DH, DH)].astype(F32)

            for j in range(4):
                beta[j] = _once(_sum((SCALE, _plus_grid_t(x_grid(j, 2), x_grid(j, 0), T[j]))))
                yield from _strassen_lhs(beta[j])
                yield from _strassen_lhs(_sum((SCALE, x_grid(j, 0))))
                for i in range(j):
                    c, d = _tau(i, j)
                    s = _sum((1, beta[i]), (1, beta[j]))
                    yield from _strassen_lhs(s)
                    for k, f in ((i, SCALE), (j, -SCALE)):
                        alpha = x_grid(k, 0)
                        if c and d:
                            grid = _sum((1, s), (c * f, _plus_grid_t(alpha, alpha, (0, c * d))))
                        else:
                            grid = _plus_grid_t(s, alpha, (c * f, d * f))
                        yield from _strassen_lhs(_once(grid))

        def q_weights(u):
            gamma = {}

            def w_grid(j, half):
                return lambda e, h: wq_bufs[half][j][
                    ((job >> 1) & 1) + zero(), u, pl.ds(e * DH, DH), pl.ds(h * DH, DH)].astype(F32)

            for j in range(4):
                yield from _strassen_rhs(w_grid(j, 1), 1)
                gamma[j] = _once(_plus_t_grid(w_grid(j, 0), (-T[j][0], -T[j][1]), w_grid(j, 1)))
                yield from _strassen_rhs(gamma[j], 0)
                for i in range(j):
                    c, d = _tau(i, j)
                    y = _once(_sum((1, gamma[i]), (1, gamma[j])))
                    if c and d:
                        w = _plus_t_grid(y, (0, -c * d), y)
                        z = _once(lambda e, h: w(e, h) * (0.5 * c))
                    elif c:
                        z = _once(lambda e, h: y(e, h) * (1 / c))
                    else:
                        z = _once(lambda e, h: y(1 - e, h) * (1 / d if e else -1 / d))
                    yield from _strassen_rhs(z, 1)
                    yield from _strassen_rhs(_sum((1, z), (1, w_grid(j, 1))), 0)
                    yield from _strassen_rhs(_sum((1, z), (-1, w_grid(i, 1))), 0)

        def q_products(u, operand):
            pp, qq = {}, {}
            first = iter(range(0, N_PRODUCTS, 7))

            def product(swap):
                n = next(first)
                return _strassen([functools.partial(operand, n + k) for k in range(7)], swap)

            def emit(i, j, c):
                for a, h in QUADS:
                    q_buf[u, 2 * i + a, 2 * j + h] = c(a, h).astype(BF16)

            for j in range(4):
                qq[j] = yield from product(1)
                pp[j] = yield from product(0)
                emit(j, j, _sum((1, pp[j]), (1, qq[j])))
                for i in range(j):
                    rr = yield from product(1)
                    uu = yield from product(0)
                    emit(i, j, _sum((1, uu), (-1, rr), (-1, pp[i]), (-1, qq[j])))
                    vv = yield from product(0)
                    emit(j, i, _sum((1, rr), (-1, vv), (-1, pp[j]), (-1, qq[i])))

        @pl.when(parity == 0)
        def _():
            todo, made = x_operands(), []

            def operand(n):
                if n == len(made):
                    made.append(next(todo)().astype(BF16))
                return made[n]

            projs = [_Projection(q_products(u, operand), q_weights(u)) for u in range(2)]
            for n, ch in enumerate(Q_PLAN):
                position[0] = n // 4
                if n in Q_WAIT:
                    k = Q_WAIT.index(n)
                    for u in range(2 if k > 0 else 0):
                        prefetch(job + 2, wq_copy, u, (k - 1) // 2, 1 - (k - 1) % 2)
                    for u in range(2 if k < 8 else 0):
                        wq_copy(0, job, u, k // 2, 1 - k % 2).wait()
                    for b in (k, k + 1) if k in (0, 2, 4, 6) else ():
                        pl.when(g == 0)(lambda: x_copy(0, b).wait())
                projs[int(ch)].step()
            assert projs[0].pending is None and projs[1].pending is None
            for u in range(2):
                q_check[u] = _column_sums(projs[u].energy) * (HS / (8 * N_PRODUCTS))

        def o_weights():
            beta = {}

            def w_grid(j, e0):
                return lambda h, e: wo_bufs[j][
                    parity + zero(), pl.ds(h * DH, DH), pl.ds((e0 + e) * DH, DH)].astype(F32)

            def diagonal(i):
                yield from _strassen_rhs(_sum((2, w_grid(i, 0))), (0, i, i) in SWAPPED)
                yield from _strassen_rhs(beta[i], (1, i, i) in SWAPPED)

            for i, j in PAIRS:
                for k in (i, j):
                    if k not in beta:
                        beta[k] = _once(_plus_grid_t(w_grid(k, 2), w_grid(k, 0), T[k]))
                c, d = _tau(i, j)
                s = _once(_sum((1, beta[i]), (1, beta[j])))
                yield from _strassen_rhs(_plus_grid_t(s, w_grid(j, 0), (-c, -d)), (1, i, j) in SWAPPED)
                yield from _strassen_rhs(_plus_grid_t(s, w_grid(i, 0), (c, d)), (1, j, i) in SWAPPED)
                yield from _strassen_rhs(s, (0, i, j) in SWAPPED)
                if j == 3:
                    yield from diagonal(i)
            yield from diagonal(3)

        def o_products():
            waiting = {(half, i): [] for half in range(2) for i in range(4)}
            started, energy = [], [None]

            def f32_grid(ref):
                return lambda a, h: ref[zero(), a, h, 0:SQ]

            def stored(slot):
                return lambda a, e: m_buf[a, e, SLOTS.index(slot), 0:SQ]

            def save(slot, grid):
                vals = {quad: grid(*quad) for quad in QUADS}
                for a, e in QUADS:
                    m_buf[a, e, SLOTS.index(slot), 0:SQ] = vals[a, e]
                return lambda a, e: vals[a, e]

            def fold(half, i, part, t):
                total = old = stored((half, i, i))
                if (half, i) not in started:
                    started.append((half, i))
                    total = lambda a, e: jnp.where(g == 0, 0.0, old(a, e))
                for grid, coef in [(part, t)] + waiting[half, i]:
                    total = _plus_grid_t(total, grid, coef)
                waiting[half, i] = []
                return save((half, i, i), total)

            def contribute(half, i, slot, part, t):
                if (half, i, slot) in FOLD_EARLY:
                    fold(half, i, part, t)
                else:
                    waiting[half, i].append((stored(slot), t))

            def diagonal(i):
                for half in range(2):
                    yield [blk for blk in BLOCKS if blk[1 - half] == i]
                    m = yield from _strassen(_strassen_lhs(f32_grid(d_bufs[2 * i + half])),
                                             (half, i, i) in SWAPPED)
                    if half == 0:
                        lo2 = fold(0, i, m, (1, 0))
                        res = [lo2(a, e) * 0.5 for a, e in QUADS]
                    else:
                        c, d = T[i]
                        minus_lo_t = [stored((0, i, i))(a, e if c else 1 - e) * (-0.5 * (c or (d if e else -d)))
                                      for a, e in QUADS]
                        hi = fold(1, i, m, (1, 0))
                        res = [hi(a, e) + v for (a, e), v in zip(QUADS, minus_lo_t)]
                    for (a, e), v in zip(QUADS, res):
                        out_buf[br, 2 * half + e, 2 * i + a] = v.astype(BF16)
                        energy.append(_sample_energy(energy[-1], v, len(energy)))
                    for e in range(2):
                        pl.when(g == NG - 1)(lambda: out_copy(br, i, 2 * half + e).start())

            for i, j in PAIRS:
                for r, k in ((i, j), (j, i)):
                    yield [(r, k)]
                    m = yield from _strassen(_strassen_lhs(f32_grid(o_bufs[r, k])), (1, r, k) in SWAPPED)
                    contribute(1, r, (1, r, k), save((1, r, k), m), (1, 0))
                diff = _sum((1, f32_grid(o_bufs[i, j])), (-1, f32_grid(o_bufs[j, i])))
                m = yield from _strassen(_strassen_lhs(diff), (0, i, j) in SWAPPED)
                ruv = save((0, i, j), _sum((1, m), (1, stored((1, j, i))), (-1, stored((1, i, j)))))
                c, d = _tau(i, j)
                for k in (i, j):
                    contribute(0, k, (0, i, j), ruv, (c, -d) if c and d else (c // 2, -d // 2))
                if j == 3:
                    yield from diagonal(i)
            yield from diagonal(3)
            out_check[br, 1] = energy[-1] * (MAX_OUT_GROWTH * N_PRODUCTS / (len(energy) - 1))

        done = []
        probs, sums, recips, least_q = {}, {}, {}, []
        pv_size = [k for ch in PLAN if ch in "Pp" for k in ((2, 2) if ch == "P" else (1,))]

        def unit(t, k):
            assert k == 1 or t % 2 == 0
            return (t // 8,) + QUADS[t // 2 % 4] + (pl.ds(t % 2 * HS, k * HS),)

        def halves(table, t, k):
            return jnp.concatenate([table[t + u] for u in range(k)], axis=0)

        def scores(t, k, back):
            n, a, h, rows = unit(t, k)
            i, j = BLOCKS[n]
            if t % 8 == 0:
                kv_copy(0, job, n, 0).wait()
            q_ref = q_buf.at[parity, 2 * i + a, 2 * j + h]
            s = lax.dot_general(q_ref[rows], k_buf[n, a, h], NT, preferred_element_type=F32)
            if t % 2 == 0:
                q = q_ref[0:HS].astype(F32)
                q = _column_sums(q * q)
                least_q.append(jnp.minimum(least_q[-1], q) if least_q else q)
            if (t + k) % 8 == 0:
                prefetch(job + 1, kv_copy, n, 0)
            e = jnp.exp2(s - jnp.max(s, axis=-1, keepdims=True))
            total = jnp.broadcast_to(jnp.sum(e, axis=-1, keepdims=True), (k * HS, DH))
            recip = pltpu.reciprocal(total, approx=True)
            for u in range(k):
                sums[t + u], recips[t + u] = total[u * HS:(u + 1) * HS], recip[u * HS:(u + 1) * HS]
            if t - back in sums:
                bound = halves(sums, t - back, k)
                bound = jnp.concatenate([bound[:8] + least_q[-1], bound[8:]], axis=0)
                e = jnp.concatenate([e[:, :SK - DH], jnp.minimum(e[:, SK - DH:], bound)], axis=-1)
            if pv_size[t] == k:
                probs[t] = e.astype(BF16)
            elif k == 2:
                probs[t], probs[t + 1] = e[:HS].astype(BF16), e[HS:].astype(BF16)
            elif t % 2 == 0:
                probs[t] = e
            else:
                probs[t - 1] = jnp.concatenate([probs[t - 1], e], axis=0).astype(BF16)

        def values(t, k):
            n, a, h, rows = unit(t, k)
            blk = BLOCKS[n]
            if t % 8 == 0:
                kv_copy(0, job, n, 1).wait()
                for j in WO_WAIT.get(n, ()):
                    wo_copy(0, job, j).wait()
                    prefetch(job + 1, wo_copy, j)
            o = jnp.dot(probs.pop(t), v_buf[n, a, h], preferred_element_type=F32)
            if (t + k) % 8 == 0:
                prefetch(job + 1, kv_copy, n, 1)
                done.append(blk)
            o = o * halves(recips, t, k)
            if blk in o_bufs:
                o_bufs[blk][0, a, h, rows] = o
            else:
                for half in range(2):
                    line = [other for other in o_bufs if other[1 - half] == blk[0]]
                    assert all(other in done for other in line)
                    d_bufs[2 * blk[0] + half][0, a, h, rows] = _lin(
                        (1, o), *[(-1, o_bufs[other][zero(), a, h, rows]) for other in line])

        proj = _Projection(o_products(), o_weights(), done)
        n_scores = n_values = 0
        for n, ch in enumerate(PLAN):
            position[0] = n + 1
            k = 2 if ch.isupper() else 1
            if ch in "STUstu":
                scores(n_scores, k, "uts".index(ch.lower()))
                n_scores += k
            elif ch in "Pp":
                values(n_values, k)
                n_values += k
            else:
                for _ in range(4 if ch == "0" else 2):
                    proj.step(1 if ch == "0" else 2)
        assert proj.pending is None and n_scores == n_values == 2 * B * G
        failed[...] += _too_large(q_check[parity], least_q[-1] * MAX_Q_GROWTH)
        out_check[br, 0] += proj.energy
        for b in range(B):
            pl.when(job == NG - 2)(lambda: x_copy(1, b).start())
        return carry

    for k in range(8):
        for u in range(2):
            wq_copy(0, 0, u, k // 2, 1 - k % 2).start()
        for b in (k, k + 1) if k % 2 == 0 else ():
            x_copy(0, b).start()
    for n in range(len(BLOCKS)):
        kv_copy(0, 0, n, 0).start()
        kv_copy(0, 0, n, 1).start()
        for j in WO_WAIT.get(n, ()):
            wo_copy(0, 0, j).start()
    check[...] = jnp.zeros(check.shape, F32)
    for i in range(4):
        for half in range(2):
            m_buf[:, :, SLOTS.index((half, i, i)), 0:SQ] = jnp.zeros((2, 2, SQ, DH), F32)
    lax.fori_loop(0, 2 * NG, run_job, 0)
    verdict = failed[...]
    for br in range(2):
        verdict += _too_large(*[
            jnp.broadcast_to(jnp.sum(_column_sums(out_check[br, n]), axis=1, keepdims=True), failed.shape)
            for n in range(2)])
    redo = jnp.max(verdict) > 0.0
    for br in range(2):
        for i in range(4):
            for e in range(4):
                out_copy(br, i, e).wait()

    def fetch(br, copy):
        for c in range(2):
            pl.when(br == c)(lambda c=c: copy(c).start())
        copy(0).wait()

    def plain_batch(n, carry):
        br, b = n >> 3, n & 7
        fetch(br, lambda c: pltpu.make_async_copy(xs[c].at[b], x_bufs[0].at[0], plain_sem))
        plain_buf[...] = jnp.zeros(plain_buf.shape, F32)

        def plain_head(h, carry):
            pair = pl.ds(pl.multiple_of((h >> 1) * 2 * DH, 2 * DH), 2 * DH)
            mine = pl.ds(pl.multiple_of((h & 1) * DH, DH), DH)
            for half in range(2):
                fetch(br, lambda c: pltpu.make_async_copy(
                    wqs[c].at[pl.ds(half * 2 * DH, 2 * DH), pair], wq_bufs[half][0].at[0, 0], plain_sem))
            fetch(br, lambda c: pltpu.make_async_copy(wos[c].at[pair, :], wo_bufs[0].at[0], plain_sem))
            fetch(br, lambda c: pltpu.make_async_copy(ks[c].at[b, h], k_buf.at[0, 0, 0], plain_sem))
            fetch(br, lambda c: pltpu.make_async_copy(vs[c].at[b, h], v_buf.at[0, 0, 0], plain_sem))
            wq = jnp.concatenate([wq_bufs[half][0][0, 0, :, mine] for half in range(2)], axis=0)
            q = jnp.dot(x_bufs[0][0], wq, preferred_element_type=F32) * SCALE
            s = lax.dot_general(q.astype(BF16), k_buf[0, 0, 0], NT, preferred_element_type=F32)
            e = jnp.exp2(s - jnp.max(s, axis=-1, keepdims=True))
            o = jnp.dot(e.astype(BF16), v_buf[0, 0, 0], preferred_element_type=F32)
            o = o / jnp.sum(e, axis=-1, keepdims=True)
            plain_buf[...] += jnp.dot(o.astype(BF16), wo_bufs[0][0, mine, :], preferred_element_type=F32)
            return carry

        lax.fori_loop(0, H, plain_head, 0)
        x_bufs[1][0] = plain_buf[...].astype(BF16)
        store = pltpu.make_async_copy(
            x_bufs[1].at[0], out_hbm.at[b, :, pl.ds(pl.multiple_of(br * D, D), D)], plain_sem)
        store.start()
        store.wait()
        return carry

    @pl.when(redo)
    def _():
        lax.fori_loop(0, 2 * B, plain_batch, 0)


@jax.jit
def pallas_concat_heads__gqa_block_cached__mha_block_cached__near_ridge_kernel(
    A_x: jax.Array,
    A_k_cache: jax.Array,
    A_v_cache: jax.Array,
    A_wq: jax.Array,
    A_wo: jax.Array,
    B_x: jax.Array,
    B_k_cache: jax.Array,
    B_v_cache: jax.Array,
    B_wq: jax.Array,
    B_wo: jax.Array,
):
    args = (A_x, A_k_cache, A_v_cache, A_wq, A_wo, B_x, B_k_cache, B_v_cache, B_wq, B_wo)
    shapes = ((B, SQ, D), (B, H, SK, DH), (B, H, SK, DH), (D, H * DH), (H * DH, D)) * 2
    assert all(a.shape == s and a.dtype == BF16 for a, s in zip(args, shapes))
    padded = SQ + 8
    hbm = pl.BlockSpec(memory_space=pl.ANY)
    return pl.pallas_call(
        _kernel,
        in_specs=[hbm] * len(args),
        out_specs=hbm,
        out_shape=jax.ShapeDtypeStruct((B, SQ, 2 * D), BF16),
        scratch_shapes=[
            pltpu.VMEM((2, B, G, SQ, DH), BF16),
            pltpu.VMEM((16, 2, 2, SK, DH), BF16),
            pltpu.VMEM((16, 2, 2, SK, DH), BF16),
            pltpu.VMEM((2, 4, B, SQ, DH), BF16),
            pltpu.VMEM((2, 2, 27, padded, DH), F32),
            pltpu.VMEM((4, 2, 8, DH), F32),
            pltpu.VMEM((SQ, D), F32),
            pltpu.SemaphoreType.DMA((60,)),
            pltpu.SemaphoreType.DMA((2, 4, 4)),
            pltpu.SemaphoreType.DMA(()),
        ]
        + [pltpu.VMEM((1, 2, 2, padded, DH), F32)] * 20
        + [pltpu.VMEM((1, SQ, D), BF16)] * 8
        + [pltpu.VMEM((2, 2, 2 * DH, 2 * DH), BF16)] * 8
        + [pltpu.VMEM((2, 2 * DH, D), BF16)] * 4,
        compiler_params=pltpu.CompilerParams(
            vmem_limit_bytes=110 * 1024 * 1024,
            disable_bounds_checks=True,
            disable_semaphore_checks=True,
            flags={"XLA_TPU_RESCHEDULE_DMA_DONES": True},
        ),
    )(*args)
```
